```python
import os as _os
_os.environ.setdefault("JAX_PLATFORMS", "cpu")
import jax
import jax.numpy as jnp

def _softmax(x, axis=-1):
    return jax.nn.softmax(x, axis=axis)
def _gelu(x):
    return jax.nn.gelu(x, approximate=True)
def _silu(x):
    return jax.nn.silu(x)
def _sigmoid(x):
    return jax.nn.sigmoid(x)
def _layernorm(x, axis=-1, eps=1e-5):
    m = jnp.mean(x, axis=axis, keepdims=True)
    v = jnp.var(x, axis=axis, keepdims=True)
    return (x - m) / jnp.sqrt(v + eps)
def _scatter_add(tgt, idx, src, axis=0):
    return tgt.at[idx].add(src)
def _segment_sum(src, seg, n):
    return jax.ops.segment_sum(src, seg, n)
class _Rng:
    def __init__(self, key):
        self._k = key
    def _next(self):
        self._k, sub = jax.random.split(self._k)
        return sub
    def normal(self, shape):
        return jax.random.normal(self._next(), shape, dtype=jnp.bfloat16)
    def randint(self, lo, hi, shape):
        return jax.random.randint(self._next(), shape, lo, hi, dtype=jnp.int32)
    def uniform(self, shape, lo=0.0, hi=1.0):
        return jax.random.uniform(self._next(), shape, jnp.bfloat16, lo, hi)
    def permutation(self, n):
        return jax.random.permutation(self._next(), n)


kernel_name = 'gated_mix__sliding_block_cached__dense_activation_silu__decode'

def setup_inputs():
    _rng = _Rng(jax.random.key(int.from_bytes(__import__("os").urandom(4), "little")))
    _w = (lambda a: (lambda t: t.astype(jnp.bfloat16) if jnp.issubdtype(t.dtype, jnp.floating) else t)(jnp.asarray(a)))
    def _A_setup():
        B, Sq, D = 2, 1, 1024
        Hq, Hkv, Sk, Dh = 32, 4, 32768, 128
        assert Hq % Hkv == 0, (Hq, Hkv)
        return {
            "x": _w((lambda *s: _rng.normal(s) * 0.05)(B, Sq, D)),
            "k_cache": _w((lambda *s: _rng.normal(s) * 3.2)(B, Hkv, Sk, Dh)),
            "v_cache": _w((lambda *s: _rng.normal(s) * 0.05)(B, Hkv, Sk, Dh)),
            "wq": _w((lambda *s: _rng.normal(s) * 3.2)(D, Hq * Dh) * (D ** -0.5)),
            "wo": _w((lambda *s: _rng.normal(s) * 0.05)(Hq * Dh, D) * ((Hq * Dh) ** -0.5)),
        }
    _A_in = _A_setup()

    def _B_setup():
        B, S, D, F = 2, 1, 1024, 3584
        return {
            "x": _w((lambda *s: _rng.normal(s) * 0.05)(B, S, D)),
            "w1": _w((lambda *s: _rng.normal(s) * 0.05)(D, F) * (D ** -0.5)),
            "w2": _w((lambda *s: _rng.normal(s) * 0.05)(F, D) * (F ** -0.5)),
        }
    _B_in = _B_setup()

    return {
        "A_x": _A_in["x"],
        "A_k_cache": _A_in["k_cache"],
        "A_v_cache": _A_in["v_cache"],
        "A_wq": _A_in["wq"],
        "A_wo": _A_in["wo"],
        "B_x": _B_in["x"],
        "B_w1": _B_in["w1"],
        "B_w2": _B_in["w2"],
        "gate_w": _w((lambda *s: _rng.normal(s) * 0.05)(1024) * 16.0),
    }

def reference(A_x, A_k_cache, A_v_cache, A_wq, A_wo, B_x, B_w1, B_w2, gate_w):
    def _A_ref(x, k_cache, v_cache, wq, wo):
        B, Sq, D = x.shape
        Hq, Dh = 32, 128
        Hkv, Sk = k_cache.shape[1], k_cache.shape[2]
        W = min(4096, max(256, Sk // 4))
        rep = Hq // Hkv
        q = (lambda x, *d: x.transpose(*d))((x @ wq).reshape(B, Sq, Hq, Dh), 0, 2, 1, 3)
        k = jnp.repeat(k_cache[:, :, Sk - W:, :], rep, axis=1)
        v = jnp.repeat(v_cache[:, :, Sk - W:, :], rep, axis=1)
        scores = jnp.einsum("bhqd,bhkd->bhqk", q, k) * (Dh ** -0.5)
        p = _softmax(scores, axis=-1)
        o = jnp.einsum("bhqk,bhkd->bhqd", p, v)
        return (lambda x, *d: x.transpose(*d))(o, 0, 2, 1, 3).reshape(B, Sq, Hq * Dh) @ wo

    def _B_ref(x, w1, w2):
        h = jnp.einsum("bsd,df->bsf", x, w1)
        h = _silu(h)
        out = jnp.einsum("bsf,fd->bsd", h, w2)
        return out

    x = A_x
    g = _sigmoid((x * gate_w).sum(-1, keepdims=True))
    a = _A_ref(x, A_k_cache, A_v_cache, A_wq, A_wo)
    b = _B_ref(x, B_w1, B_w2)
    return g * a + (1 - g) * b
```

```python
import functools

import jax
import jax.numpy as jnp
import jax.experimental.pallas as pl
import jax.experimental.pallas.tpu as pltpu

_BF = jnp.bfloat16
_F32 = jnp.float32

DEPTH = 4
LAST = 1


def _kernel(x_hbm, k_hbm, v_hbm, wq_hbm, wo_hbm, w1_hbm, w2_hbm, g_hbm, o_hbm,
            xb, gb, wqb, kb, vb, w1b, w2b, wob,
            xs, qacc, qg, pbuf, lbuf, og, ow, hacc, hs, ob,
            sems, msem, *, B, Hq, Hkv, Sk, W, Dh, D, F, depth):
  rep = Hq // Hkv
  NG = B * Hkv
  RQ = 128
  RO = 512
  nq = D // RQ
  n1 = D // RQ
  n2 = F // RO
  no = (Hq * Dh) // RO
  scale = Dh ** -0.5

  def c_wq(i, s):
    r = pl.ds(pl.multiple_of(i * RQ, RQ), RQ)
    return pltpu.make_async_copy(wq_hbm.at[r], wqb.at[r], sems.at[s])

  def c_k(i, s):
    return pltpu.make_async_copy(
        k_hbm.at[i // Hkv, i % Hkv, pl.ds(Sk - W, W)], kb.at[i], sems.at[s])

  def c_v(i, s):
    return pltpu.make_async_copy(
        v_hbm.at[i // Hkv, i % Hkv, pl.ds(Sk - W, W)], vb.at[i], sems.at[s])

  def c_w1(i, s):
    r = pl.ds(pl.multiple_of(i * RQ, RQ), RQ)
    return pltpu.make_async_copy(w1_hbm.at[r], w1b.at[r], sems.at[s])

  def c_w2(i, s):
    r = pl.ds(pl.multiple_of(i * RO, RO), RO)
    return pltpu.make_async_copy(w2_hbm.at[r], w2b.at[r], sems.at[s])

  def c_wo(i, s):
    r = pl.ds(pl.multiple_of(i * RO, RO), RO)
    return pltpu.make_async_copy(wo_hbm.at[r], wob.at[r], sems.at[s])

  phases = [(c_wq, nq), (c_k, NG), (c_v, NG), (c_w1, n1), (c_w2, n2), (c_wo, no)]
  base = [0]
  for _, n in phases:
    base.append(base[-1] + n)
  assert all(n >= depth for _, n in phases)

  def step(p, i):
    fn, n = phases[p]
    fn(i, base[p] + i).wait()
    j = i + depth

    @pl.when(j < n)
    def _():
      fn(j, base[p] + j).start()

    if p + 1 < len(phases):
      @pl.when(j >= n)
      def _():
        phases[p + 1][0](j - n, base[p] + j).start()

  for i in range(depth):
    c_wq(i, i).start()
    if i == 0:
      cx = pltpu.make_async_copy(x_hbm, xb, msem.at[0])
      cg = pltpu.make_async_copy(g_hbm, gb, msem.at[1])
      cx.start()
      cg.start()
  cx.wait()
  cg.wait()

  xf = xb[...].astype(_F32)
  gf = gb[...].astype(_F32)
  row = jax.lax.broadcasted_iota(jnp.int32, (8, 128), 0)
  gsum = jnp.zeros((8, 128), _F32)
  for j in range(D // 128):
    blk = xf[:, j * 128:(j + 1) * 128]
    t = jnp.zeros((8, 128), _F32)
    for b in range(B):
      t = jnp.where(row == b, jnp.broadcast_to(blk[b:b + 1, :], (8, 128)), t)
    xs[j] = t.astype(_BF)
    gsum = gsum + t * gf[j:j + 1, :]
  gate = jax.nn.sigmoid(jnp.sum(gsum, axis=-1, keepdims=True))

  qacc[...] = jnp.zeros(qacc.shape, _F32)

  def q_body(i, c):
    step(0, i)
    r = pl.ds(pl.multiple_of(i * RQ, RQ), RQ)
    qacc[...] += jnp.dot(xs[i], wqb[r, :], preferred_element_type=_F32)
    return c
  jax.lax.fori_loop(0, nq, q_body, 0)

  for g in range(Hkv):
    tiles = [qacc[:, (g * rep + r) * Dh:(g * rep + r + 1) * Dh] for r in range(rep)]
    for b in range(B):
      t = jnp.zeros((8, 128), _F32)
      for r in range(rep):
        t = jnp.where(row == r, jnp.broadcast_to(tiles[r][b:b + 1, :], (8, 128)), t)
      qg[b * Hkv + g] = t.astype(_BF)

  def k_body(i, c):
    step(1, i)
    s = jax.lax.dot_general(qg[i], kb[i], (((1,), (1,)), ((), ())),
                            preferred_element_type=_F32) * scale
    m = jnp.max(s, axis=-1, keepdims=True)
    p = jnp.exp(s - m)
    lbuf[i] = jnp.broadcast_to(jnp.sum(p, axis=-1, keepdims=True), (8, 128))
    pbuf[i] = p.astype(_BF)
    return c
  jax.lax.fori_loop(0, NG, k_body, 0)

  def v_body(i, c):
    step(2, i)
    og[i] = jnp.dot(pbuf[i], vb[i], preferred_element_type=_F32) / lbuf[i]
    return c
  jax.lax.fori_loop(0, NG, v_body, 0)

  hp = RO // Dh
  for g in range(Hkv):
    ts = [og[b * Hkv + g] for b in range(B)]
    for r in range(rep):
      h = g * rep + r
      t = jnp.zeros((8, 128), _F32)
      for b in range(B):
        t = jnp.where(row == b, jnp.broadcast_to(ts[b][r:r + 1, :], (8, 128)), t)
      ow[h // hp, :, (h % hp) * Dh:(h % hp + 1) * Dh] = t.astype(_BF)

  hacc[...] = jnp.zeros(hacc.shape, _F32)

  def h_body(i, c):
    step(3, i)
    r = pl.ds(pl.multiple_of(i * RQ, RQ), RQ)
    hacc[...] += jnp.dot(xs[i], w1b[r, :], preferred_element_type=_F32)
    return c
  jax.lax.fori_loop(0, n1, h_body, 0)

  for j in range(n2):
    hv = hacc[:, j * RO:(j + 1) * RO]
    hs[j] = (hv * jax.nn.sigmoid(hv)).astype(_BF)

  def b_body(i, acc):
    step(4, i)
    r = pl.ds(pl.multiple_of(i * RO, RO), RO)
    return acc + jnp.dot(hs[i], w2b[r, :], preferred_element_type=_F32)
  bacc = jax.lax.fori_loop(0, n2, b_body, jnp.zeros((8, D), _F32))

  def a_body(i, acc):
    step(5, i)
    r = pl.ds(pl.multiple_of(i * RO, RO), RO)
    return acc + jnp.dot(ow[i], wob[r, :], preferred_element_type=_F32)
  aacc = jax.lax.fori_loop(0, no, a_body, jnp.zeros((8, D), _F32))

  res = gate * aacc + (1.0 - gate) * bacc
  ob[...] = res[0:B, :].astype(_BF)
  co = pltpu.make_async_copy(ob, o_hbm, msem.at[2])
  co.start()
  co.wait()


def build(depth=DEPTH):
  def fn(A_x, A_k_cache, A_v_cache, A_wq, A_wo, B_x, B_w1, B_w2, gate_w):
    B, Sq, D = A_x.shape
    assert Sq == 1
    Hq, Dh = 32, 128
    Hkv, Sk = A_k_cache.shape[1], A_k_cache.shape[2]
    W = min(4096, max(256, Sk // 4))
    F = B_w1.shape[1]
    NG = B * Hkv
    kern = functools.partial(_kernel, B=B, Hq=Hq, Hkv=Hkv, Sk=Sk, W=W, Dh=Dh,
                             D=D, F=F, depth=depth)
    V = pltpu.VMEM
    out = pl.pallas_call(
        kern,
        in_specs=[pl.BlockSpec(memory_space=pl.ANY)] * 8,
        out_specs=pl.BlockSpec(memory_space=pl.ANY),
        out_shape=jax.ShapeDtypeStruct((B, D), _BF),
        scratch_shapes=[
            V((B, D), _BF), V((D // 128, 128), _BF),
            V((D, Hq * Dh), _BF), V((NG, W, Dh), _BF), V((NG, W, Dh), _BF),
            V((D, F), _BF), V((F, D), _BF), V((Hq * Dh, D), _BF),
            V((D // 128, 8, 128), _BF), V((8, Hq * Dh), _F32),
            V((NG, 8, Dh), _BF), V((NG, 8, W), _BF), V((NG, 8, 128), _F32),
            V((NG, 8, Dh), _F32), V((Hq * Dh // 512, 8, 512), _BF),
            V((8, F), _F32), V((F // 512, 8, 512), _BF), V((B, D), _BF),
            pltpu.SemaphoreType.DMA((64,)), pltpu.SemaphoreType.DMA((3,)),
        ],
        compiler_params=pltpu.CompilerParams(vmem_limit_bytes=64 * 2**20),
    )(A_x.reshape(B, D), A_k_cache, A_v_cache, A_wq, A_wo, B_w1, B_w2,
      gate_w.reshape(D // 128, 128))
    return out.reshape(B, 1, D)
  return fn


@jax.jit
def pallas_gated_mix__sliding_block_cached__dense_activation_silu__decode_kernel(
    A_x, A_k_cache, A_v_cache, A_wq, A_wo, B_x, B_w1, B_w2, gate_w):
  return build()(A_x, A_k_cache, A_v_cache, A_wq, A_wo, B_x, B_w1, B_w2, gate_w)
```

```python
import functools

import jax
import jax.numpy as jnp
import jax.experimental.pallas as pl
import jax.experimental.pallas.tpu as pltpu

_BF = jnp.bfloat16
_F32 = jnp.float32


def _kernel(x_hbm, k_hbm, v_hbm, wq_hbm, wo_hbm, w1_hbm, w2_hbm, g_hbm, o_hbm,
            xb, gb, wqb, kb, vb, w1b, w2b, wob,
            xs, qacc, qg, pbuf, lbuf, og, ow, hacc, hs, ob,
            sems, msem, *, B, Hq, Hkv, Sk, W, Dh, D, F, wo_split, alt, xprio, depth):
  rep = Hq // Hkv
  NG = B * Hkv
  RQ = 128
  RO = 512
  nq = D // RQ
  n1 = D // RQ
  n2 = F // RO
  no = (Hq * Dh) // RO
  scale = Dh ** -0.5

  copies = []

  def add(src, dst):
    i = len(copies)
    copies.append(pltpu.make_async_copy(src, dst, sems.at[i]))
    return _Chunk(i)

  def start(i):
    copies[i].start(priority=(i % 2 if alt else 0))

  class _Chunk:
    def __init__(self, i):
      self.i = i

    def wait(self):
      copies[self.i].wait()
      if self.i + depth < len(copies):
        start(self.i + depth)

  c_wq = add(wq_hbm, wqb)
  c_k = add(k_hbm.at[:, :, pl.ds(Sk - W, W)], kb)
  c_v = add(v_hbm.at[:, :, pl.ds(Sk - W, W)], vb)
  c_w1 = add(w1_hbm, w1b)
  c_w2 = add(w2_hbm, w2b)
  c_wo = {}
  r0 = 0
  for n in wo_split:
    c_wo[r0] = add(wo_hbm.at[pl.ds(r0, n)], wob.at[pl.ds(r0, n)])
    r0 += n
  assert r0 == Hq * Dh

  cx = pltpu.make_async_copy(x_hbm, xb, msem.at[0])
  cg = pltpu.make_async_copy(g_hbm, gb, msem.at[1])
  for i in range(min(depth, len(copies))):
    start(i)
    if i == 0:
      cx.start(priority=xprio)
      cg.start(priority=xprio)
  cx.wait()
  cg.wait()

  xf = xb[...].astype(_F32)
  gf = gb[...].astype(_F32)
  row = jax.lax.broadcasted_iota(jnp.int32, (8, 128), 0)
  gsum = jnp.zeros((8, 128), _F32)
  for j in range(D // 128):
    blk = xf[:, j * 128:(j + 1) * 128]
    t = jnp.zeros((8, 128), _F32)
    for b in range(B):
      t = jnp.where(row == b, jnp.broadcast_to(blk[b:b + 1, :], (8, 128)), t)
    xs[j] = t.astype(_BF)
    gsum = gsum + t * gf[j:j + 1, :]
  gate = jax.nn.sigmoid(jnp.sum(gsum, axis=-1, keepdims=True))

  qacc[...] = jnp.zeros(qacc.shape, _F32)

  def q_body(i, c):
    r = pl.ds(pl.multiple_of(i * RQ, RQ), RQ)
    qacc[...] += jnp.dot(xs[i], wqb[r, :], preferred_element_type=_F32)
    return c
  c_wq.wait()
  jax.lax.fori_loop(0, nq, q_body, 0)

  for g in range(Hkv):
    tiles = [qacc[:, (g * rep + r) * Dh:(g * rep + r + 1) * Dh] for r in range(rep)]
    for b in range(B):
      t = jnp.zeros((8, 128), _F32)
      for r in range(rep):
        t = jnp.where(row == r, jnp.broadcast_to(tiles[r][b:b + 1, :], (8, 128)), t)
      qg[b * Hkv + g] = t.astype(_BF)

  def k_body(i, c):
    s = jax.lax.dot_general(qg[i], kb[i // Hkv, i % Hkv], (((1,), (1,)), ((), ())),
                            preferred_element_type=_F32) * scale
    m = jnp.max(s, axis=-1, keepdims=True)
    p = jnp.exp(s - m)
    lbuf[i] = jnp.broadcast_to(jnp.sum(p, axis=-1, keepdims=True), (8, 128))
    pbuf[i] = p.astype(_BF)
    return c
  c_k.wait()
  jax.lax.fori_loop(0, NG, k_body, 0)

  def v_body(i, c):
    og[i] = jnp.dot(pbuf[i], vb[i // Hkv, i % Hkv], preferred_element_type=_F32) / lbuf[i]
    return c
  c_v.wait()
  jax.lax.fori_loop(0, NG, v_body, 0)

  hp = RO // Dh
  for g in range(Hkv):
    ts = [og[b * Hkv + g] for b in range(B)]
    for r in range(rep):
      h = g * rep + r
      t = jnp.zeros((8, 128), _F32)
      for b in range(B):
        t = jnp.where(row == b, jnp.broadcast_to(ts[b][r:r + 1, :], (8, 128)), t)
      ow[h // hp, :, (h % hp) * Dh:(h % hp + 1) * Dh] = t.astype(_BF)

  hacc[...] = jnp.zeros(hacc.shape, _F32)

  def h_body(i, c):
    r = pl.ds(pl.multiple_of(i * RQ, RQ), RQ)
    hacc[...] += jnp.dot(xs[i], w1b[r, :], preferred_element_type=_F32)
    return c
  c_w1.wait()
  jax.lax.fori_loop(0, n1, h_body, 0)

  for j in range(n2):
    hv = hacc[:, j * RO:(j + 1) * RO]
    hs[j] = (hv * jax.nn.sigmoid(hv)).astype(_BF)

  def b_body(i, acc):
    r = pl.ds(pl.multiple_of(i * RO, RO), RO)
    return acc + jnp.dot(hs[i], w2b[r, :], preferred_element_type=_F32)
  c_w2.wait()
  bacc = jax.lax.fori_loop(0, n2, b_body, jnp.zeros((8, D), _F32))

  bacc = (1.0 - gate) * bacc
  nfull = 0
  for n in wo_split:
    if n % RO:
      break
    nfull += n // RO

  def a_body(i, acc):
    for r0, c in c_wo.items():
      if r0 < nfull * RO:
        pl.when(i == r0 // RO)(c.wait)
    r = pl.ds(pl.multiple_of(i * RO, RO), RO)
    return acc + jnp.dot(ow[i], wob[r, :], preferred_element_type=_F32)
  aacc = jax.lax.fori_loop(0, nfull, a_body, jnp.zeros((8, D), _F32))
  for (r0, c), n in zip(c_wo.items(), wo_split):
    if r0 >= nfull * RO:
      assert r0 % RO + n <= RO
      c.wait()
      aacc = aacc + jnp.dot(ow[r0 // RO, :, r0 % RO:r0 % RO + n],
                            wob[r0:r0 + n, :], preferred_element_type=_F32)

  res = gate * aacc + bacc
  ob[...] = res[0:B, :].astype(_BF)
  co = pltpu.make_async_copy(ob, o_hbm, msem.at[2])
  co.start()
  co.wait()


def build(wo_split=(2048, 1024, 512, 256, 128, 128), alt=True, xprio=0, depth=3):
  def fn(A_x, A_k_cache, A_v_cache, A_wq, A_wo, B_x, B_w1, B_w2, gate_w):
    B, Sq, D = A_x.shape
    assert Sq == 1
    Hq, Dh = 32, 128
    Hkv, Sk = A_k_cache.shape[1], A_k_cache.shape[2]
    W = min(4096, max(256, Sk // 4))
    F = B_w1.shape[1]
    NG = B * Hkv
    kern = functools.partial(_kernel, B=B, Hq=Hq, Hkv=Hkv, Sk=Sk, W=W, Dh=Dh,
                             D=D, F=F, wo_split=wo_split, alt=alt, xprio=xprio, depth=depth)
    V = pltpu.VMEM
    out = pl.pallas_call(
        kern,
        in_specs=[pl.BlockSpec(memory_space=pl.ANY)] * 8,
        out_specs=pl.BlockSpec(memory_space=pl.ANY),
        out_shape=jax.ShapeDtypeStruct((B, D), _BF),
        scratch_shapes=[
            V((B, D), _BF), V((D // 128, 128), _BF),
            V((D, Hq * Dh), _BF), V((B, Hkv, W, Dh), _BF), V((B, Hkv, W, Dh), _BF),
            V((D, F), _BF), V((F, D), _BF), V((Hq * Dh, D), _BF),
            V((D // 128, 8, 128), _BF), V((8, Hq * Dh), _F32),
            V((NG, 8, Dh), _BF), V((NG, 8, W), _BF), V((NG, 8, 128), _F32),
            V((NG, 8, Dh), _F32), V((Hq * Dh // 512, 8, 512), _BF),
            V((8, F), _F32), V((F // 512, 8, 512), _BF), V((B, D), _BF),
            pltpu.SemaphoreType.DMA((5 + len(wo_split),)), pltpu.SemaphoreType.DMA((3,)),
        ],
        compiler_params=pltpu.CompilerParams(vmem_limit_bytes=64 * 2**20),
    )(A_x.reshape(B, D), A_k_cache, A_v_cache, A_wq, A_wo, B_w1, B_w2,
      gate_w.reshape(D // 128, 128))
    return out.reshape(B, 1, D)
  return fn


@jax.jit
def pallas_gated_mix__sliding_block_cached__dense_activation_silu__decode_kernel(
    A_x, A_k_cache, A_v_cache, A_wq, A_wo, B_x, B_w1, B_w2, gate_w):
  return build()(A_x, A_k_cache, A_v_cache, A_wq, A_wo, B_x, B_w1, B_w2, gate_w)
```
